```python
import jax
import jax.numpy as jnp

def _softmax(x, axis=-1):
    return jax.nn.softmax(x, axis=axis)
def _gelu(x):
    return jax.nn.gelu(x, approximate=True)
def _silu(x):
    return jax.nn.silu(x)
def _sigmoid(x):
    return jax.nn.sigmoid(x)
def _layernorm(x, axis=-1, eps=1e-5):
    m = jnp.mean(x, axis=axis, keepdims=True)
    v = jnp.var(x, axis=axis, keepdims=True)
    return (x - m) / jnp.sqrt(v + eps)
def _scatter_add(tgt, idx, src, axis=0):
    return tgt.at[idx].add(src)
def _segment_sum(src, seg, n):
    return jax.ops.segment_sum(src, seg, n)
class _Rng:
    def __init__(self, key):
        self._k = key
    def _next(self):
        self._k, sub = jax.random.split(self._k)
        return sub
    def normal(self, shape):
        return jax.random.normal(self._next(), shape, dtype=jnp.bfloat16)
    def randint(self, lo, hi, shape):
        return jax.random.randint(self._next(), shape, lo, hi, dtype=jnp.int32)
    def uniform(self, shape, lo=0.0, hi=1.0):
        return jax.random.uniform(self._next(), shape, jnp.bfloat16, lo, hi)
    def permutation(self, n):
        return jax.random.permutation(self._next(), n)


kernel_name = 'standalone__cross_network_dcn__recsys'

def setup_inputs():
    _rng = _Rng(jax.random.key(int.from_bytes(__import__("os").urandom(4), "little")))
    _w = (lambda a: (lambda t: t.astype(jnp.bfloat16) if jnp.issubdtype(t.dtype, jnp.floating) else t)(jnp.asarray(a)))
    B, F, D, L = 16384, 100, 16, 6
    Din = min(F * D, 1024)
    return {
        "x0": _w((lambda *s: _rng.normal(s) * 0.05)(B, Din)),
        "ws": _w((lambda *s: _rng.normal(s) * 0.05)(L, Din, Din) * (Din ** -0.5)),
        "bs": _w((lambda *s: _rng.normal(s) * 0.05)(L, Din) * 0.01),
    }

def reference(x0, ws, bs):
    x = x0
    L = ws.shape[0]
    for l in range(L):
        proj = jnp.einsum('bd,de->be', x, ws[l]) + bs[l]
        x = x0 * proj + x
    return x
```

```python
import jax
import jax.numpy as jnp
import jax.experimental.pallas as pl
import jax.experimental.pallas.tpu as pltpu

_BM = 512
_SUB = 256


def _cross_kernel(x0_ref, w_ref, b_ref, o_ref):
    n_layers = w_ref.shape[0]
    n_sub = _BM // _SUB
    x0 = [x0_ref[pl.ds(s * _SUB, _SUB), :] for s in range(n_sub)]
    x = list(x0)
    for l in range(n_layers):
        b = b_ref[pl.ds(l, 1), :].astype(jnp.float32)
        for s in range(n_sub):
            proj = jnp.dot(x[s], w_ref[l], preferred_element_type=jnp.float32) + b
            x[s] = (x0[s].astype(jnp.float32) * proj
                    + x[s].astype(jnp.float32)).astype(o_ref.dtype)
    for s in range(n_sub):
        o_ref[pl.ds(s * _SUB, _SUB), :] = x[s]


@jax.jit
def pallas_standalone__cross_network_dcn__recsys_kernel(
    x0: jax.Array,
    ws: jax.Array,
    bs: jax.Array,
):
    batch, d = x0.shape
    n_layers = ws.shape[0]
    return pl.pallas_call(
        _cross_kernel,
        grid=(batch // _BM,),
        in_specs=[
            pl.BlockSpec((_BM, d), lambda i: (i, 0)),
            pl.BlockSpec((n_layers, d, d), lambda i: (0, 0, 0),
                         pipeline_mode=pl.Buffered(1)),
            pl.BlockSpec((n_layers, d), lambda i: (0, 0)),
        ],
        out_specs=pl.BlockSpec((_BM, d), lambda i: (i, 0)),
        out_shape=jax.ShapeDtypeStruct((batch, d), x0.dtype),
        compiler_params=pltpu.CompilerParams(
            dimension_semantics=("arbitrary",),
            vmem_limit_bytes=100 * 1024 * 1024,
        ),
    )(x0, ws, bs)
```

```python
import functools

import jax
import jax.numpy as jnp
import jax.experimental.pallas as pl
import jax.experimental.pallas.tpu as pltpu

_F32 = jnp.float32
_BF16 = jnp.bfloat16

_TILE = 512
_PLAIN_TILE = 256
_PAD = 16

_LHS = {1: ((0, 1), (3, 1)), 2: ((2, 1), (3, 1)), 3: ((0, 1),), 4: ((3, 1),),
        5: ((0, 1), (1, 1)), 6: ((2, 1), (0, -1)), 7: ((1, 1), (3, -1))}
_RHS = {1: ((0, 1), (3, 1)), 2: ((0, 1),), 3: ((1, 1), (3, -1)),
        4: ((2, 1), (0, -1)), 5: ((3, 1),), 6: ((0, 1), (1, 1)),
        7: ((2, 1), (3, 1))}
_OUT = {0: {1: 1, 4: 1, 5: -1, 7: 1}, 1: {3: 1, 5: 1}, 2: {2: 1, 4: 1},
        3: {1: 1, 2: -1, 3: 1, 6: 1}}
_ORDER = (3, 5, 4, 2, 1, 7, 6)
_N_PARTIAL = 7
_SUMS = (1, 2, 5, 6, 7)
_EAGER_SUMS = (1, 2, 5, 6)
_SCAN_AT = ((1, 1), (1, 2), (2, 1), (2, 2))


def _signed_sum(terms, get):
    total = get(terms[0][0])
    for quadrant, sign in terms[1:]:
        total = total + get(quadrant) if sign > 0 else total - get(quadrant)
    return total


class _OutputSums:
    def __init__(self, keep):
        self._keep = keep
        self._partial = {}
        self._missing = {c: len(uses) for c, uses in _OUT.items()}

    def add(self, m, product):
        finished, kept = [], None
        for c, uses in _OUT.items():
            if m not in uses:
                continue
            self._missing[c] -= 1
            if c not in self._partial:
                kept = kept or self._keep(product)
                self._partial[c] = (kept, uses[m])
                continue
            get, sign = self._partial[c]
            if sign < 0:
                assert uses[m] > 0
                total = product - get()
            else:
                total = get() + product if uses[m] > 0 else get() - product
            if self._missing[c]:
                self._partial[c] = (self._keep(total), 1)
            else:
                finished.append((c, total))
        return finished


def _rounding_ok(x0_max, w_sq, b_max):
    return ((3200.0 * (x0_max * x0_max) * w_sq <= 1.0)
            & ((x0_max + 1.0) * (b_max + 1.0) <= 1e15)).astype(jnp.int32)


def _cross_kernel(x0_hbm, w_hbm, b_hbm, o_hbm,
                  x0_buf, o_buf, w_ref, wp_ref, b_in, b_ref, px0_ref, px_ref,
                  x_sem, o_sem, w_sem, sem, *blocks):
    n_layers, d, _ = w_ref.shape
    n_tiles = x0_hbm.shape[0] // _TILE
    bh, bw = _TILE // 4, d // 4
    n_part = 4 * _N_PARTIAL
    part_blocks, x_blocks, sum_blocks = (
        blocks[:n_part], blocks[n_part:n_part + 32], blocks[n_part + 32:])

    def rows(p, q):
        return pl.ds((p // 2 * 2 + q // 2) * bh, bh)

    def cols(p, q):
        return pl.ds((p % 2 * 2 + q % 2) * bw, bw)

    def tile(t):
        return pl.ds(pl.multiple_of(t * _TILE, _TILE), _TILE)

    def x_copy(t):
        return pltpu.make_async_copy(
            x0_hbm.at[tile(jnp.minimum(t, n_tiles - 1))], x0_buf.at[t & 3],
            x_sem.at[t & 3])

    def o_copy(t):
        return pltpu.make_async_copy(
            o_buf.at[t & 1], o_hbm.at[tile(t)], o_sem.at[t & 1])

    def w_copy(l):
        return pltpu.make_async_copy(w_hbm.at[l], w_ref.at[l], w_sem.at[l])

    b_copy = pltpu.make_async_copy(b_hbm, b_in, sem.at[0])
    for l in range(n_layers):
        w_copy(l).start()
    b_copy.start()
    x_copy(0).start()
    x_copy(1).start()

    def prepare_layer(l, w_sq):
        w_copy(l).wait()
        for c in range(0, bw, 128):
            def prepare_rows(j, squares, c=c):
                r = pl.multiple_of(j * 16, 16)
                w = {(p, q): w_ref[l, pl.ds(r + (p // 2 * 2 + q // 2) * bw, 16),
                                   pl.ds(cols(p, q).start + c, 128)].astype(_F32)
                     for p in range(4) for q in range(4)}
                for m in _RHS:
                    outer = [_signed_sum(_RHS[m], lambda p, q=q: w[p, q])
                             for q in range(4)]
                    for n in _RHS:
                        rhs = _signed_sum(_RHS[n], outer.__getitem__)
                        wp_ref[l, 7 * (m - 1) + n - 1,
                               pl.ds(pl.multiple_of(j * 8, 8), 8),
                               pl.ds(c, 128)] = pltpu.bitcast(
                                   rhs.astype(_BF16), jnp.int32)
                return [s + (v * v).reshape(2, 8, 128).sum(0)
                        for s, v in zip(squares, w.values())]

            for s in jax.lax.fori_loop(0, bw // 16, prepare_rows,
                                       [jnp.zeros((8, 128), _F32)] * 16):
                w_sq = jnp.maximum(w_sq, jnp.sum(s, axis=0, keepdims=True))
        return w_sq

    w_sq = jnp.max(jax.lax.fori_loop(0, n_layers, prepare_layer,
                                     jnp.zeros((1, 128), _F32)))
    b_copy.wait()
    b_ref[...] = b_in[...].astype(_F32)
    b_max = jnp.max(jnp.abs(b_ref[...]))

    def scan(slot, p, q):
        v = jnp.abs(x0_buf[slot, rows(p, q), cols(p, q)].astype(_F32))
        return jnp.max(v.reshape(bh // 8, 8, bw), axis=0)

    def check(scans):
        return _rounding_ok(jnp.max(functools.reduce(jnp.maximum, scans)),
                            w_sq, b_max)

    def strassen_tile(state):
        t, _ = state
        zero = t >> 30
        x_copy(t + 1).wait()
        x_copy(t + 2).start()

        @pl.when(t >= 2)
        def _():
            o_copy(t - 2).wait()

        x_done, sums_done, scanned = set(), set(), []

        def x0_block(p, q):
            return x0_buf[t & 3, rows(p, q), cols(p, q)]

        def x_ref(l, p, q):
            return x_blocks[l % 2 * 16 + 4 * p + q]

        def x_block(l, p, q, at=zero):
            if l == 0:
                return x0_block(p, q).astype(_F32)
            return x_ref(l, p, q)[at, 0:bh]

        def sum_ref(l, m, q):
            return sum_blocks[(l % 2 * len(_SUMS) + _SUMS.index(m)) * 4 + q]

        def outer_lhs(l, m, q):
            if l == 0 or m not in _SUMS:
                return _signed_sum(_LHS[m], lambda p: x_block(l, p, q))
            if (l, m, q) not in sums_done:
                sum_ref(l, m, q)[0] = _signed_sum(
                    _LHS[m], lambda p: x_block(l, p, q))
                sums_done.add((l, m, q))
            return sum_ref(l, m, q)[zero]

        def lhs(l, m, n):
            if l == 0 and m not in _SUMS and n not in _SUMS:
                return x0_block(_LHS[m][0][0], _LHS[n][0][0])
            return _signed_sum(
                _LHS[n], lambda q: outer_lhs(l, m, q)).astype(_BF16)

        def store_x(l, p, q, value):
            x_ref(l, p, q)[0, 0:bh] = value
            x_done.add((l, p, q))
            for m in _EAGER_SUMS:
                if ((l, m, q) not in sums_done
                        and all((l, u, q) in x_done for u, _ in _LHS[m])):
                    sum_ref(l, m, q)[0] = _signed_sum(
                        _LHS[m],
                        lambda u: value if u == p else x_block(l, u, q))
                    sums_done.add((l, m, q))

        def keep_in(refs):
            free = list(refs)

            def keep(value):
                ref = free.pop(0)
                ref[0] = value
                return lambda: ref[zero]
            return keep

        for l in range(n_layers):
            last = l == n_layers - 1
            if last:
                next_ok = check([ref[zero, bh:bh + 8] for ref in scanned])
            outer_sums = [
                _OutputSums(keep_in(
                    part_blocks[q * _N_PARTIAL:(q + 1) * _N_PARTIAL]))
                for q in range(4)]
            for m in _ORDER:
                inner_sums = _OutputSums(lambda value: lambda: value)
                for n in _ORDER:
                    product = jnp.dot(
                        lhs(l, m, n),
                        pltpu.bitcast(wp_ref[l, 7 * (m - 1) + n - 1], _BF16),
                        preferred_element_type=_F32)
                    for q, inner in inner_sums.add(n, product):
                        for p, proj in outer_sums[q].add(m, inner):
                            x = x_block(l, p, q, next_ok >> 1 if (
                                last and (p, q) == (1, 0)) else zero)
                            x = x0_block(p, q).astype(_F32) * (
                                proj + b_ref[l:l + 1, cols(p, q)]) + x
                            if last:
                                o_buf[t & 1, rows(p, q), cols(p, q)] = (
                                    x.astype(o_buf.dtype))
                                continue
                            store_x(l + 1, p, q, x)
                            if (l, p) in _SCAN_AT:
                                scanned.append(x_ref(l + 1, p, q))
                                scanned[-1][0, bh:bh + 8] = scan(
                                    (t + 1) & 3, _SCAN_AT.index((l, p)), q)
        o_copy(t).start()
        return t + 1, next_ok

    x_copy(0).wait()
    first_ok = check([scan(0, p, q) for p in range(4) for q in range(4)])
    done, _ = jax.lax.while_loop(
        lambda state: (state[0] < n_tiles) & (state[1] != 0),
        strassen_tile, (jnp.int32(0), first_ok))

    x_copy(done + 1).wait()
    for back in (2, 1):
        @pl.when(done >= back)
        def _(back=back):
            o_copy(done - back).wait()

    def plain_tile(t, carry):
        at = pl.ds(pl.multiple_of(t * _PLAIN_TILE, _PLAIN_TILE), _PLAIN_TILE)
        load = pltpu.make_async_copy(x0_hbm.at[at], px0_ref, sem.at[0])
        load.start()
        load.wait()
        px_ref[...] = px0_ref[...].astype(_F32)

        def layer(l, carry):
            x = px_ref[...]
            proj = jnp.dot(x.astype(_BF16), w_ref[l],
                           preferred_element_type=_F32) + b_ref[pl.ds(l, 1), :]
            px_ref[...] = px0_ref[...].astype(_F32) * proj + x
            return carry

        jax.lax.fori_loop(0, n_layers, layer, 0)
        px0_ref[...] = px_ref[...].astype(px0_ref.dtype)
        store = pltpu.make_async_copy(px0_ref, o_hbm.at[at], sem.at[0])
        store.start()
        store.wait()
        return carry

    per_tile = _TILE // _PLAIN_TILE
    jax.lax.fori_loop(done * per_tile, n_tiles * per_tile, plain_tile, 0)


@jax.jit
def pallas_standalone__cross_network_dcn__recsys_kernel(
    x0: jax.Array,
    ws: jax.Array,
    bs: jax.Array,
):
    batch, d = x0.shape
    n_layers = ws.shape[0]
    assert batch % _TILE == 0 and d % 512 == 0 and 4 <= n_layers <= 6
    assert x0.dtype == ws.dtype == bs.dtype == _BF16
    bh, bw = _TILE // 4, d // 4
    hbm = pl.BlockSpec(memory_space=pl.ANY)
    return pl.pallas_call(
        _cross_kernel,
        in_specs=[hbm, hbm, hbm],
        out_specs=hbm,
        out_shape=jax.ShapeDtypeStruct((batch, d), x0.dtype),
        scratch_shapes=[
            pltpu.VMEM((4, _TILE, d), _BF16),
            pltpu.VMEM((2, _TILE, d), _BF16),
            pltpu.VMEM((n_layers, d, d), _BF16),
            pltpu.VMEM((n_layers, 49, bw // 2, bw), jnp.int32),
            pltpu.VMEM((n_layers, d), _BF16),
            pltpu.VMEM((n_layers, d), _F32),
            pltpu.VMEM((_PLAIN_TILE, d), _BF16),
            pltpu.VMEM((_PLAIN_TILE, d), _F32),
            pltpu.SemaphoreType.DMA((4,)),
            pltpu.SemaphoreType.DMA((2,)),
            pltpu.SemaphoreType.DMA((n_layers,)),
            pltpu.SemaphoreType.DMA((1,)),
        ]
        + [pltpu.VMEM((1, bh, bw), _F32)] * (4 * _N_PARTIAL)
        + [pltpu.VMEM((1, bh + _PAD, bw), _F32)] * 32
        + [pltpu.VMEM((1, bh, bw), _F32)] * (2 * len(_SUMS) * 4),
        compiler_params=pltpu.CompilerParams(
            vmem_limit_bytes=100 * 1024 * 1024),
    )(x0, ws, bs)
```

```python
import jax
import jax.numpy as jnp
import jax.experimental.pallas as pl
import jax.experimental.pallas.tpu as pltpu

_TILE = 512


def _cross_layer(x0, x, w, b):
    proj = jnp.dot(x, w, preferred_element_type=jnp.float32) + b
    return (x0.astype(jnp.float32) * proj
            + x.astype(jnp.float32)).astype(x.dtype)


def _cross_kernel(x0_hbm, w_hbm, b_in, o_hbm,
                  x0_buf, o_buf, w_ref, b_ref, x_sem, o_sem, w_sem):
    n_layers = w_ref.shape[0]
    n_tiles = x0_hbm.shape[0] // _TILE

    def tile(t):
        return pl.ds(pl.multiple_of(t * _TILE, _TILE), _TILE)

    def x_copy(t):
        return pltpu.make_async_copy(
            x0_hbm.at[tile(jnp.minimum(t, n_tiles - 1))], x0_buf.at[t & 1],
            x_sem.at[t & 1])

    def o_copy(t):
        return pltpu.make_async_copy(
            o_buf.at[t & 1], o_hbm.at[tile(t)], o_sem.at[t & 1])

    def w_copy(l):
        return pltpu.make_async_copy(w_hbm.at[l], w_ref.at[l], w_sem.at[l])

    x_copy(0).start()
    w_copy(0).start()
    b_ref[...] = b_in[...].astype(jnp.float32)
    x_copy(0).wait()
    o_buf[0] = x0_buf[0]

    def first_tile_layer(l, carry):
        w_copy(l).wait()

        @pl.when(l + 1 < n_layers)
        def _():
            w_copy(l + 1).start()

        @pl.when(l + 1 == n_layers)
        def _():
            x_copy(1).start()

        o_buf[0] = _cross_layer(
            x0_buf[0], o_buf[0], w_ref[l], b_ref[pl.ds(l, 1), :])
        return carry

    jax.lax.fori_loop(0, n_layers, first_tile_layer, 0)
    o_copy(0).start()

    def other_tile(t, carry):
        x_copy(t).wait()
        x_copy(t + 1).start()

        @pl.when(t >= 2)
        def _():
            o_copy(t - 2).wait()

        x = x0 = x0_buf[t & 1]
        for l in range(n_layers):
            x = _cross_layer(x0, x, w_ref[l], b_ref[l:l + 1, :])
        o_buf[t & 1] = x
        o_copy(t).start()
        return carry

    jax.lax.fori_loop(1, n_tiles, other_tile, 0)

    x_copy(n_tiles).wait()
    for t in range(max(n_tiles - 2, 0), n_tiles):
        o_copy(t).wait()


@jax.jit
def pallas_standalone__cross_network_dcn__recsys_kernel(
    x0: jax.Array,
    ws: jax.Array,
    bs: jax.Array,
):
    batch, d = x0.shape
    n_layers = ws.shape[0]
    assert batch % _TILE == 0
    hbm = pl.BlockSpec(memory_space=pl.ANY)
    return pl.pallas_call(
        _cross_kernel,
        in_specs=[hbm, hbm, pl.BlockSpec(memory_space=pltpu.VMEM)],
        out_specs=hbm,
        out_shape=jax.ShapeDtypeStruct((batch, d), x0.dtype),
        scratch_shapes=[
            pltpu.VMEM((2, _TILE, d), x0.dtype),
            pltpu.VMEM((2, _TILE, d), x0.dtype),
            pltpu.VMEM((n_layers, d, d), ws.dtype),
            pltpu.VMEM((n_layers, d), jnp.float32),
            pltpu.SemaphoreType.DMA((2,)),
            pltpu.SemaphoreType.DMA((2,)),
            pltpu.SemaphoreType.DMA((n_layers,)),
        ],
        compiler_params=pltpu.CompilerParams(
            vmem_limit_bytes=64 * 1024 * 1024),
    )(x0, ws, bs)
```
